```python
import jax
import jax.numpy as jnp

def _softmax(x, axis=-1):
    return jax.nn.softmax(x, axis=axis)
def _gelu(x):
    return jax.nn.gelu(x, approximate=True)
def _silu(x):
    return jax.nn.silu(x)
def _sigmoid(x):
    return jax.nn.sigmoid(x)
def _layernorm(x, axis=-1, eps=1e-5):
    m = jnp.mean(x, axis=axis, keepdims=True)
    v = jnp.var(x, axis=axis, keepdims=True)
    return (x - m) / jnp.sqrt(v + eps)
def _scatter_add(tgt, idx, src, axis=0):
    return tgt.at[idx].add(src)
def _segment_sum(src, seg, n):
    return jax.ops.segment_sum(src, seg, n)
class _Rng:
    def __init__(self, key):
        self._k = key
    def _next(self):
        self._k, sub = jax.random.split(self._k)
        return sub
    def normal(self, shape):
        return jax.random.normal(self._next(), shape, dtype=jnp.bfloat16)
    def randint(self, lo, hi, shape):
        return jax.random.randint(self._next(), shape, lo, hi, dtype=jnp.int32)
    def uniform(self, shape, lo=0.0, hi=1.0):
        return jax.random.uniform(self._next(), shape, jnp.bfloat16, lo, hi)
    def permutation(self, n):
        return jax.random.permutation(self._next(), n)


kernel_name = 'concat_heads__ssm_conv_s5__sliding_local_dilated__prompt'

def setup_inputs():
    _rng = _Rng(jax.random.key(int.from_bytes(__import__("os").urandom(4), "little")))
    _w = (lambda a: (lambda t: t.astype(jnp.bfloat16) if jnp.issubdtype(t.dtype, jnp.floating) else t)(jnp.asarray(a)))
    def _A_setup():
        B, S, D = 1, 2048, 448
        P = D
        Lambda_re = -0.5 * jnp.exp((lambda *s: _rng.normal(s) * 0.05)(P))
        Lambda_im = (lambda *s: _rng.normal(s) * 0.05)(P) * 1.0
        B_re = (lambda *s: _rng.normal(s) * 0.05)(P, D) * (D ** -0.5)
        B_im = (lambda *s: _rng.normal(s) * 0.05)(P, D) * (D ** -0.5)
        C_re = (lambda *s: _rng.normal(s) * 0.05)(D, P) * (P ** -0.5)
        C_im = (lambda *s: _rng.normal(s) * 0.05)(D, P) * (P ** -0.5)
        log_dt = (lambda *s: _rng.normal(s) * 0.05)(P) * 0.3 - 2.0
        Dskip = (lambda *s: _rng.normal(s) * 0.05)(D)
        return {
            "x": _w((lambda *s: _rng.normal(s) * 0.05)(B, S, D)),
            "Lambda_re": _w(Lambda_re),
            "Lambda_im": _w(Lambda_im),
            "B_re": _w(B_re),
            "B_im": _w(B_im),
            "C_re": _w(C_re),
            "C_im": _w(C_im),
            "log_dt": _w(log_dt),
            "Dskip": _w(Dskip),
        }
    _A_in = _A_setup()

    def _B_setup():
        B, S, D = 1, 2048, 448
        return {
            "x": _w((lambda *s: _rng.normal(s) * 0.05)(B, S, D)),
            "wqkv": _w((lambda *s: _rng.normal(s) * 0.05)(D, 3 * D)),
            "wo": _w((lambda *s: _rng.normal(s) * 0.05)(D, D)),
        }
    _B_in = _B_setup()

    return {
        "A_x": _A_in["x"],
        "A_Lambda_re": _A_in["Lambda_re"],
        "A_Lambda_im": _A_in["Lambda_im"],
        "A_B_re": _A_in["B_re"],
        "A_B_im": _A_in["B_im"],
        "A_C_re": _A_in["C_re"],
        "A_C_im": _A_in["C_im"],
        "A_log_dt": _A_in["log_dt"],
        "A_Dskip": _A_in["Dskip"],
        "B_x": _B_in["x"],
        "B_wqkv": _B_in["wqkv"],
        "B_wo": _B_in["wo"],
    }

def reference(A_x, A_Lambda_re, A_Lambda_im, A_B_re, A_B_im, A_C_re, A_C_im, A_log_dt, A_Dskip, B_x, B_wqkv, B_wo):
    def _A_ref(x, Lambda_re, Lambda_im, B_re, B_im, C_re, C_im, log_dt, Dskip):
        Bsz, L, H = x.shape
        Lam = Lambda_re + 1j * Lambda_im
        Bmat = B_re + 1j * B_im
        Cmat = C_re + 1j * C_im
        dt = jnp.exp(log_dt)
        Lam_bar = jnp.exp(dt * Lam)
        B_bar = ((Lam_bar - 1.0) / Lam)[:, None] * Bmat
        Bu = jnp.einsum("bld,pd->blp", x + 0j, B_bar)
        h = jnp.zeros_like(Bu[:, 0, :])
        hs = []
        for t in range(L):
            h = Lam_bar[None, :] * h + Bu[:, t, :]
            hs.append(h)
        hseq = jnp.stack(hs, 1)
        y = 2.0 * jnp.einsum("blp,dp->bld", hseq, Cmat).real + x * Dskip[None, None, :]
        return y

    def _B_ref(x, wqkv, wo):
        B, S, D = x.shape
        H = 16; Dh = D // H
        W, dil = 8, 2
        qkv = (lambda x, *d: x.transpose(*d))((x @ wqkv).reshape(B, S, 3, H, Dh), 2, 0, 3, 1, 4)
        q, k, v = qkv[0], qkv[1], qkv[2]
        scale = Dh ** -0.5
        pos = jnp.arange(S)
        off = jnp.arange(W) * dil
        idx = pos[:, None] - off[None, :]
        mask = idx >= 0
        idx_c = jnp.where(mask, idx, 0).reshape(-1)
        kg = k[:, :, idx_c, :].reshape(B, H, S, W, Dh)
        vg = v[:, :, idx_c, :].reshape(B, H, S, W, Dh)
        logits = jnp.einsum("bhsd,bhswd->bhsw", q, kg) * scale
        logits = jnp.where(mask[None, None, :, :], logits, -1e9)
        attn = _softmax(logits, axis=-1)
        o = jnp.einsum("bhsw,bhswd->bhsd", attn, vg)
        return (lambda x, *d: x.transpose(*d))(o, 0, 2, 1, 3).reshape(B, S, D) @ wo

    a = _A_ref(A_x, A_Lambda_re, A_Lambda_im, A_B_re, A_B_im, A_C_re, A_C_im, A_log_dt, A_Dskip)
    b = _B_ref(B_x, B_wqkv, B_wo)
    return jnp.concatenate([a, b], axis=-1)
```

```python
import jax
import jax.numpy as jnp
from jax import lax
import jax.experimental.pallas as pl
import jax.experimental.pallas.tpu as pltpu

F32 = jnp.float32
BF16 = jnp.bfloat16

S = 2048
D = 448
H = 16
DH = D // H
W = 8
DIL = 2
T = 512
G = T // 128
L = T // 8
LP = L + 4
NDP = DH // 2
HALO = 16


def _nt(a, b):
    return lax.dot_general(a, b, (((1,), (1,)), ((), ())), preferred_element_type=F32)


def _nn(a, b):
    return jnp.dot(a, b, preferred_element_type=F32)


def _cmul(ar, ai, br, bi):
    return ar * br - ai * bi, ar * bi + ai * br


def _kernel(lre_ref, lim_ref, ldt_ref, dsk_ref, xa_ref, xb_ref, bre_ref, bim_ref,
            cre_ref, cim_ref, wqkv_ref, wo_ref, out_ref,
            wqt, wot, bcat, ccat, dcol, lam, carry, bu, stage, qs, ks, vs, tail, ot, wof):
    step = pl.program_id(0)
    lane = lax.broadcasted_iota(jnp.int32, (8, 128), 1)
    sub = lax.broadcasted_iota(jnp.int32, (8, 128), 0)

    @pl.when(step == 0)
    def _prep():
        lr = lre_ref[...].astype(F32).reshape(1, D)
        li = lim_ref[...].astype(F32).reshape(1, D)
        dt = jnp.exp(ldt_ref[...].astype(F32).reshape(1, D)).astype(BF16).astype(F32)
        mag = jnp.exp(dt * lr)
        ar = mag * jnp.cos(dt * li)
        ai = mag * jnp.sin(dt * li)
        nr, ni = ar - 1.0, ai
        big = jnp.abs(lr) >= jnp.abs(li)
        r = jnp.where(big, li / lr, lr / li)
        den = jnp.where(big, lr + li * r, lr * r + li)
        fr = 2.0 * jnp.where(big, nr + ni * r, nr * r + ni) / den
        fi = 2.0 * jnp.where(big, ni - nr * r, ni * r - nr) / den
        cr = cre_ref[...].astype(F32)
        ci = cim_ref[...].astype(F32)
        er, ei = _cmul(cr, ci, fr, fi)
        ccat[:, 0:384] = er[:, 0:384].astype(BF16)
        ccat[:, 384:768] = (-ei[:, 0:384]).astype(BF16)
        ccat[:, 768:896] = jnp.concatenate([er[:, 384:], -ei[:, 384:]], axis=1).astype(BF16)
        bcat[0:384] = bre_ref[0:384]
        bcat[384:768] = bim_ref[0:384]
        bcat[768:832] = bre_ref[384:448]
        bcat[832:896] = bim_ref[384:448]
        for j in range(4):
            if j < 3:
                pr, pi = ar[:, j * 128:(j + 1) * 128], ai[:, j * 128:(j + 1) * 128]
            else:
                pr = jnp.concatenate([ar[:, 384:], ar[:, 384:]], axis=1)
                pi = jnp.concatenate([ai[:, 384:], -ai[:, 384:]], axis=1)
            pr = jnp.broadcast_to(pr, (8, 128))
            pi = jnp.broadcast_to(pi, (8, 128))
            lam[0, j], lam[1, j] = pr, pi
            for _ in range(L.bit_length() - 1):
                pr, pi = _cmul(pr, pi, pr, pi)
            for k in range(3):
                lam[2 + 2 * k, j], lam[3 + 2 * k, j] = pr, pi
                pr, pi = _cmul(pr, pi, pr, pi)
        carry[...] = jnp.zeros(carry.shape, F32)
        tail[...] = jnp.zeros(tail.shape, F32)
        dsk = jnp.broadcast_to(dsk_ref[...].astype(F32).reshape(1, D), (128, D))
        dcol[...] = dsk.T
        wqt[...] = wqkv_ref[...].T
        wo = wo_ref[...].astype(F32)
        for j in range(4):
            wd = 128 if j < 3 else 64
            wof[j, :, 0:wd] = wo[:, j * 128:j * 128 + wd]
        for j in range(4):
            wd = 128 if j < 3 else 64
            rows = [wof[j, pl.ds(d + 8 * u * DH, 8, stride=DH), :]
                    for d in range(DH) for u in range(2)]
            wot[j * 128:j * 128 + wd, :] = jnp.concatenate(rows, axis=0).T[0:wd].astype(BF16)

    for g in range(G):
        stage[g] = _nn(wqt[...], xb_ref[:, g * 128:(g + 1) * 128])
    for which, dst in enumerate((qs, ks, vs)):
        for dp in range(NDP):
            pieces = [stage[g, pl.ds(which * D + 2 * dp + e + 8 * u * DH, 8, stride=DH), :]
                      for e in range(2) for g in range(G) for u in range(2)]
            t = jnp.concatenate(pieces, axis=0).T
            if which == 0:
                dst[dp] = t
            else:
                dst[dp, HALO:] = t
                lane16 = lax.broadcasted_iota(jnp.int32, (HALO, 128), 1)
                first = pltpu.roll(tail[which - 1, dp], 128 - 48, 1)
                if which == 2:
                    first = jnp.where(step == 0, jnp.broadcast_to(t[0:1], (HALO, 128)), first)
                cur = t[128 - HALO:]
                dst[dp, 0:HALO] = jnp.where((lane16 % 64) < 16, first, pltpu.roll(cur, 16, 1))
                tail[which - 1, dp] = cur

    xa = xa_ref[...].T
    u = _nt(xa, bcat[...])
    for j in range(7):
        for c in range(8):
            bu[j, pl.ds(c * LP, L), :] = u[c * L:(c + 1) * L, j * 128:(j + 1) * 128]
    for c in range(8):
        bu[7, pl.ds(c * LP, L), :] = pltpu.roll(u[c * L:(c + 1) * L, 768:896], 64, 1)

    for j in range(4):
        jr, ji = (j, j + 3) if j < 3 else (6, 7)
        pr, pi = lam[0, j], lam[1, j]
        hr = bu[jr, pl.ds(0, 8, stride=LP), :]
        hi = bu[ji, pl.ds(0, 8, stride=LP), :]
        for r in range(1, L):
            mr, mi = _cmul(pr, pi, hr, hi)
            hr = mr + bu[jr, pl.ds(r, 8, stride=LP), :]
            hi = mi + bu[ji, pl.ds(r, 8, stride=LP), :]
        hr = pltpu.roll(jnp.where(sub == 7, carry[0, j], hr), 1, 0)
        hi = pltpu.roll(jnp.where(sub == 7, carry[1, j], hi), 1, 0)
        for k in range(3):
            sr = jnp.where(sub >= (1 << k), pltpu.roll(hr, 1 << k, 0), 0.0)
            si = jnp.where(sub >= (1 << k), pltpu.roll(hi, 1 << k, 0), 0.0)
            mr, mi = _cmul(lam[2 + 2 * k, j], lam[3 + 2 * k, j], sr, si)
            hr, hi = hr + mr, hi + mi
        for r in range(L):
            mr, mi = _cmul(pr, pi, hr, hi)
            hr = mr + bu[jr, pl.ds(r, 8, stride=LP), :]
            hi = mi + bu[ji, pl.ds(r, 8, stride=LP), :]
            bu[jr, pl.ds(r, 8, stride=LP), :] = hr
            if j < 3:
                bu[ji, pl.ds(r, 8, stride=LP), :] = hi
        carry[0, j], carry[1, j] = hr, hi

    scale = DH ** -0.5
    for rg in range(16):
        r0 = rg * 8
        acc = [None] * W
        for dp in range(NDP):
            q = qs[dp, r0:r0 + 8]
            for w in range(W):
                p = q * ks[dp, pl.ds(HALO + r0 - DIL * w, 8), :]
                acc[w] = p if dp == 0 else acc[w] + p
        lg = [(a + pltpu.roll(a, 64, 1)) * scale for a in acc]
        for w in range(W):
            if r0 - DIL * w < 0:
                bad = (step == 0) & ((lane % 64) < 16) & (sub + (r0 - DIL * w) < 0)
                lg[w] = jnp.where(bad, -1e9, lg[w])
        m = lg[0]
        for w in range(1, W):
            m = jnp.maximum(m, lg[w])
        ex = [jnp.exp(x - m) for x in lg]
        tot = ex[0]
        for w in range(1, W):
            tot = tot + ex[w]
        inv = 1.0 / tot
        ex = [x * inv for x in ex]
        for dp in range(NDP):
            o = ex[0] * vs[dp, pl.ds(HALO + r0, 8), :]
            for w in range(1, W):
                o = o + ex[w] * vs[dp, pl.ds(HALO + r0 - DIL * w, 8), :]
            qs[dp, r0:r0 + 8] = o
    for dp in range(NDP):
        t = qs[dp].T
        for e in range(2):
            for g in range(G):
                ot[pl.ds((2 * dp + e) * H, H), g * 128:(g + 1) * 128] = (
                    t[(e * G + g) * H:(e * G + g + 1) * H].astype(BF16))

    h = jnp.concatenate(
        [jnp.concatenate([bu[j, pl.ds(c * LP, L), :] for c in range(8)], axis=0)
         for j in range(7)], axis=1).astype(BF16)
    y = _nt(ccat[...], h)
    b = _nn(wot[...], ot[...])
    for g in range(G):
        cols = slice(g * 128, (g + 1) * 128)
        a = y[:, cols] + xa_ref[:, cols].astype(F32) * dcol[...]
        out_ref[cols, :] = jnp.concatenate([a, b[:, cols]], axis=0).T


@jax.jit
def pallas_concat_heads__ssm_conv_s5__sliding_local_dilated__prompt_kernel(
    A_x: jax.Array,
    A_Lambda_re: jax.Array,
    A_Lambda_im: jax.Array,
    A_B_re: jax.Array,
    A_B_im: jax.Array,
    A_C_re: jax.Array,
    A_C_im: jax.Array,
    A_log_dt: jax.Array,
    A_Dskip: jax.Array,
    B_x: jax.Array,
    B_wqkv: jax.Array,
    B_wo: jax.Array,
):
    whole = lambda shape: pl.BlockSpec(shape, lambda i: (0,) * len(shape))
    xspec = pl.BlockSpec((D, T), lambda i: (0, i))
    out = pl.pallas_call(
        _kernel,
        grid=(S // T,),
        in_specs=[whole((D,))] * 4 + [xspec, xspec] + [whole((D, D))] * 4
        + [whole((D, 3 * D)), whole((D, D))],
        out_specs=pl.BlockSpec((T, 2 * D), lambda i: (i, 0)),
        out_shape=jax.ShapeDtypeStruct((S, 2 * D), F32),
        scratch_shapes=[
            pltpu.VMEM((3 * D, D), BF16),
            pltpu.VMEM((D, D), BF16),
            pltpu.VMEM((2 * D, D), BF16),
            pltpu.VMEM((D, 2 * D), BF16),
            pltpu.VMEM((D, 128), F32),
            pltpu.VMEM((8, 4, 8, 128), F32),
            pltpu.VMEM((2, 4, 8, 128), F32),
            pltpu.VMEM((8, 8 * LP, 128), F32),
            pltpu.VMEM((G, 3 * D, 128), F32),
            pltpu.VMEM((NDP, 128, 128), F32),
            pltpu.VMEM((NDP, HALO + 128, 128), F32),
            pltpu.VMEM((NDP, HALO + 128, 128), F32),
            pltpu.VMEM((2, NDP, HALO, 128), F32),
            pltpu.VMEM((D, T), BF16),
            pltpu.VMEM((4, D, 128), F32),
        ],
        compiler_params=pltpu.CompilerParams(
            dimension_semantics=("arbitrary",), vmem_limit_bytes=100 << 20),
        name="s5_dilated_attn",
    )(A_Lambda_re, A_Lambda_im, A_log_dt, A_Dskip,
      jnp.swapaxes(A_x[0], 0, 1), jnp.swapaxes(B_x[0], 0, 1),
      A_B_re, A_B_im, A_C_re, A_C_im, B_wqkv, B_wo)
    return out[None]
```

```python
import functools

import jax
import jax.numpy as jnp
from jax import lax
import jax.experimental.pallas as pl
import jax.experimental.pallas.tpu as pltpu

F32 = jnp.float32
BF16 = jnp.bfloat16
U32 = jnp.uint32

S = 2048
D = 448
H = 16
DH = D // H
W = 8
DIL = 2
T = 512
NB = S // T
G = T // 128
L = T // 8
LP = L + 4
NDP = DH // 2
HALO = 16
LAG = 5
LAG_END = 1
SCAN_STEP = 16
KT = ((0, 128), (128, 128), (256, 128), (384, 64))
PIECES = ((0, 8, 0, 7),) + tuple((t, 1, 0, 7) for t in range(8, 15)) + (
    (15, 1, 0, 3), (15, 1, 3, 2), (15, 1, 5, 2))
ORDER = ("A0 A1 B0 B1 A2 Y0 Y1 O0 O1 B2 A3 B3 Y20 O20 Y21 O21 Y22 O22 Y23 O23 "
         "Y30 Y31 O30 O31 Y32 O32 Y33 O33")
ATT = 130
AHEAD = 1
QUIET = 600


def _nt(a, b):
    return lax.dot_general(a, b, (((1,), (1,)), ((), ())), preferred_element_type=F32)


def _nn(a, b):
    return jnp.dot(a, b, preferred_element_type=F32)


def _cmul(ar, ai, br, bi):
    return ar * br - ai * bi, ar * bi + ai * br


def _pack(x):
    return pltpu.bitcast(x.astype(BF16), U32)


def _wide(ref, width):
    n = -(-width // 128)
    x = jnp.concatenate([pltpu.bitcast(ref[j], BF16) for j in range(n)], axis=1)
    return x[:, 0:width]


def _kernel(lre_hbm, lim_hbm, ldt_hbm, dsk_hbm, xa_hbm, xb_hbm, bre_hbm, bim_hbm,
            cre_hbm, cim_hbm, wqkv_hbm, wo_hbm, out_hbm,
            vec, xa_v, xb_v, bcat, cre_v, cim_v, wqkv_v, wo_v, out_v,
            wqt, wot, ccat, dcol, lam, coef, wof, isem, osem, bu, stage, qs, ks, vs, ot, xat, outt):
    lane = lax.broadcasted_iota(jnp.int32, (8, 128), 1)
    sub = lax.broadcasted_iota(jnp.int32, (8, 128), 0)

    copies = {}

    def add(name, src, dst, sem=None):
        sem = isem.at[len(copies)] if sem is None else sem
        copies[name] = pltpu.make_async_copy(src, dst, sem)

    for n, src in enumerate((lre_hbm, lim_hbm, ldt_hbm, dsk_hbm)):
        add(f"v{n}", src, vec[n])
    add("b0", bre_hbm.at[0:256], bcat.at[0:256])
    add("b4", bre_hbm.at[256:384], bcat.at[256:384])
    add("b1", bim_hbm.at[0:384], bcat.at[384:768])
    add("b2", bre_hbm.at[384:448], bcat.at[768:832])
    add("b3", bim_hbm.at[384:448], bcat.at[832:896])
    add("wqkv", wqkv_hbm, wqkv_v)
    add("cre", cre_hbm, cre_v)
    add("cim", cim_hbm, cim_v)
    add("wo", wo_hbm, wo_v)
    for i in range(NB):
        add(f"xa{i}", xa_hbm.at[:, pl.ds(i * T, T)], xa_v[i])
        add(f"xb{i}", xb_hbm.at[:, pl.ds(i * T, T)], xb_v[i])
    for p, (t0, nt, j0, nj) in enumerate(PIECES):
        add(f"o{p}", out_v[p].at[0:nt * 128],
            out_hbm.at[pl.ds(t0 * 128, nt * 128), pl.ds(j0 * 128, nj * 128)],
            osem.at[p])

    def dma(start="", wait=""):
        for n in start.split():
            copies[n].start()
        for n in wait.split():
            copies[n].wait()

    val = {}

    def prep_lambda():
        lr = vec[0][...].astype(F32).reshape(1, D)
        li = vec[1][...].astype(F32).reshape(1, D)
        dt = jnp.exp(vec[2][...].astype(F32).reshape(1, D)).astype(BF16).astype(F32)
        mag = jnp.exp(dt * lr)
        ar = mag * jnp.cos(dt * li)
        ai = mag * jnp.sin(dt * li)
        nr, ni = ar - 1.0, ai
        big = jnp.abs(lr) >= jnp.abs(li)
        r = jnp.where(big, li / lr, lr / li)
        den = jnp.where(big, lr + li * r, lr * r + li)
        fr = 2.0 * jnp.where(big, nr + ni * r, nr * r + ni) / den
        fi = 2.0 * jnp.where(big, ni - nr * r, ni * r - nr) / den
        for j in range(4):
            if j < 3:
                pr, pi, qr, qi = (v[:, j * 128:(j + 1) * 128] for v in (ar, ai, fr, fi))
            else:
                pr = jnp.concatenate([ar[:, 384:], ar[:, 384:]], axis=1)
                pi = jnp.concatenate([ai[:, 384:], -ai[:, 384:]], axis=1)
                qr = jnp.concatenate([fr[:, 384:], -fr[:, 384:]], axis=1)
                qi = jnp.concatenate([fi[:, 384:], fi[:, 384:]], axis=1)
            coef[0, j], coef[1, j] = jnp.broadcast_to(qr, (8, 128)), jnp.broadcast_to(qi, (8, 128))
            pr = jnp.broadcast_to(pr, (8, 128))
            pi = jnp.broadcast_to(pi, (8, 128))
            lam[0, j], lam[1, j] = pr, pi
            for _ in range(L.bit_length() - 1):
                pr, pi = _cmul(pr, pi, pr, pi)
            for k in range(3):
                lam[2 + 2 * k, j], lam[3 + 2 * k, j] = pr, pi
                pr, pi = _cmul(pr, pi, pr, pi)
        a = jnp.broadcast_to(lr[:, 0:128], (8, 128))
        b = jnp.broadcast_to(li[:, 0:128], (8, 128))
        val["never"] = (a > b) & (b > a)

    def prep_skip():
        dsk = jnp.broadcast_to(vec[3][...].astype(F32).reshape(1, D), (128, D))
        dcol[...] = dsk.T

    last = {}
    marks = []

    def after(stream, x):
        return jnp.where(val["never"], last[stream], x) if stream in last else x

    def released(x):
        return jnp.where(val["never"], val["mxu"], x)

    def paced(rhs):
        marks.append(dict(last))
        lag = LAG if len(marks) < len(mxu) - 8 else LAG_END
        if len(marks) <= lag:
            return rhs
        old = marks[-lag - 2] if len(marks) > lag + 1 else {}
        deps = [v for k, v in marks[-lag - 1].items() if old.get(k) is not v]
        if not deps:
            return rhs
        head = pltpu.bitcast(rhs[0:16, 0:128], F32)
        for v in deps:
            head = jnp.where(val["never"], v, head)
        head = pltpu.bitcast(head, BF16)
        if rhs.shape[1] > 128:
            head = jnp.concatenate([head, rhs[0:16, 128:]], axis=1)
        return jnp.concatenate([head, rhs[16:]], axis=0)

    def prep_c(j, r0):
        cols = slice(KT[j][0], KT[j][0] + KT[j][1])
        for r in range(r0, r0 + 64, 16):
            cr, ci = cre_v[r:r + 16, cols].astype(F32), cim_v[r:r + 16, cols].astype(F32)
            if j == 3:
                cr, ci = jnp.concatenate([cr, ci], axis=1), jnp.concatenate([ci, cr], axis=1)
            fr = after("prep", coef[0, j])
            fi = after("prep", coef[1, j])
            if r == r0:
                fr = released(fr)
            fr, fi = (jnp.concatenate([v, v], axis=0) for v in (fr, fi))
            half = slice(r // 2, r // 2 + 8)
            ccat[6 if j == 3 else j, half] = done = _pack(cr * fr - ci * fi)
            if j < 3:
                ccat[3 + j, half] = done = _pack(-(cr * fi + ci * fr))
            last["prep"] = pltpu.bitcast(done, F32)

    def prep_wqkv(j):
        k0, wd = KT[j]
        w = wqkv_v[k0:k0 + wd, :]
        if wd < 128:
            w = jnp.concatenate([w, jnp.zeros((128 - wd, 3 * D), BF16)], axis=0)
        wqt[j] = _pack(w.T)

    def prep_wo(j):
        n0, wd = KT[j]
        w = wo_v[:, n0:n0 + wd].astype(F32)
        if wd < 128:
            w = jnp.concatenate([w, jnp.zeros((D, 128 - wd), F32)], axis=1)
        wof[j] = jnp.concatenate([released(w[r:r + 8]) for r in range(0, D, 8)], axis=0)
        for k, (k0, kw) in enumerate(KT):
            rows = [wof[j, pl.ds(d + 8 * u * DH, 8, stride=DH), :]
                    for d in range(k0 // H, (k0 + kw) // H) for u in range(2)]
            if kw < 128:
                rows.append(jnp.zeros((128 - kw, 128), F32))
            t = jnp.concatenate(rows, axis=0).T
            wot[k, n0 // 2:(n0 + wd) // 2] = _pack(t[0:wd])
        last["prep"] = t[0:8]

    def xt(i, j):
        k0, wd = KT[j]
        x = xa_v[i][k0:k0 + wd, :]
        if wd < 128:
            x = jnp.concatenate([x, jnp.zeros((128 - wd, T), BF16)], axis=0)
        xat[i][j] = _pack(x.T)

    def a1(i, j):
        u = _nt(_wide(xat[i], D), paced(bcat[j * 128:(j + 1) * 128]))
        val["mxu"] = u[0:8]
        for c in range(8):
            bu[i][j][pl.ds(c * LP, L), :] = u[c * L:(c + 1) * L]

    def swap(i):
        for c in range(8):
            bu[i][7][pl.ds(c * LP, L), :] = pltpu.roll(bu[i][6][pl.ds(c * LP, L), :], 64, 1)

    carry = [(0.0, 0.0)] * 4
    state = [None] * 4

    def a2(i, j, second, r0):
        jr, ji = (j, j + 3) if j < 3 else (6, 7)
        pr, pi = lam[0, j], lam[1, j]
        if second and r0 == 0:
            hr, hi = state[j]
            cr, ci = carry[j]
            hr = pltpu.roll(jnp.where(sub == 7, cr, hr), 1, 0)
            hi = pltpu.roll(jnp.where(sub == 7, ci, hi), 1, 0)
            for k in range(3):
                sr = jnp.where(sub >= (1 << k), pltpu.roll(hr, 1 << k, 0), 0.0)
                si = jnp.where(sub >= (1 << k), pltpu.roll(hi, 1 << k, 0), 0.0)
                mr, mi = _cmul(lam[2 + 2 * k, j], lam[3 + 2 * k, j], sr, si)
                hr, hi = hr + mr, hi + mi
            state[j] = hr, hi
        for r in range(r0, r0 + SCAN_STEP):
            ur = bu[i][jr][pl.ds(r, 8, stride=LP), :]
            ui = bu[i][ji][pl.ds(r, 8, stride=LP), :]
            if r == 0 and not second:
                state[j] = released(after("scan", ur)), after("scan", ui)
                continue
            mr, mi = _cmul(pr, pi, *state[j])
            state[j] = hr, hi = mr + ur, mi + ui
            if second:
                bu[i][jr][pl.ds(r, 8, stride=LP), :] = hr
                if j < 3:
                    bu[i][ji][pl.ds(r, 8, stride=LP), :] = hi
        if second and r0 + SCAN_STEP == L:
            carry[j] = state[j]
        last["scan"] = state[j][0]

    def b1(i, n, g):
        w = _wide(wqt.at[:, n * D // 2:(n + 1) * D // 2], D)
        u = _nn(w, paced(xb_v[i][:, g * 128:(g + 1) * 128]))
        val["mxu"] = u[0:8]
        stage[i][g, n * D:(n + 1) * D] = u

    def restack(i, which, dp):
        dst = (qs, ks, vs)[which]
        half = lax.broadcasted_iota(jnp.int32, (HALO, 128), 1) % 64
        pieces = [stage[i][g, pl.ds(which * D + 2 * dp + e + 8 * u * DH, 8, stride=DH), :]
                  for e in range(2) for g in range(G) for u in range(2)]
        t = jnp.concatenate(pieces, axis=0).T
        last["xlu"] = t[120:128]
        if which == 0:
            dst[i][dp] = t
            return
        dst[i][dp, HALO:] = t
        if i == 0:
            first = jnp.broadcast_to(t[0:1], (HALO, 128))
        else:
            first = pltpu.roll(dst[i - 1][dp, 128:], 128 - 48, 1)
        dst[i][dp, 0:HALO] = jnp.where(half < 16, first, pltpu.roll(t[128 - HALO:], 16, 1))

    logits = {}

    def scores(i, r0):
        lg = []
        for w in range(W):
            for dp in range(NDP):
                t = qs[i][dp, r0:r0 + 8] * ks[i][dp, pl.ds(HALO + r0 - DIL * w, 8), :]
                a = after("qk", t) if dp == 0 else a + t
                if dp == 0 and w == 0:
                    a = after("pv", a)
            last["qk"] = a
            a = (a + pltpu.roll(a, 64, 1)) * DH ** -0.5
            if i == 0 and r0 - DIL * w < 0:
                bad = ((lane % 64) < 16) & (sub + (r0 - DIL * w) < 0)
                a = jnp.where(bad, -1e9, a)
            lg.append(a)
        m = functools.reduce(jnp.maximum, lg)
        ex = [jnp.exp(x - m) for x in lg]
        inv = 1.0 / functools.reduce(jnp.add, ex)
        logits[i, r0] = [x * inv for x in ex]

    def blend(i, r0):
        ex = logits.pop((i, r0))
        for dp in range(NDP):
            o = after("pv", ex[0] * vs[i][dp, pl.ds(HALO + r0, 8), :])
            for w in range(1, W):
                o = o + ex[w] * vs[i][dp, pl.ds(HALO + r0 - DIL * w, 8), :]
            last["pv"] = o
            qs[i][dp, r0:r0 + 8] = o

    def unstack(i, dp):
        t = qs[i][dp].T
        last["xlu"] = t[120:128]
        for e in range(2):
            for g in range(G):
                ot[i][g, pl.ds((2 * dp + e) * H // 2, H // 2), :] = _pack(
                    t[(e * G + g) * H:(e * G + g + 1) * H])

    def a3(i, g):
        h = jnp.concatenate(
            [jnp.concatenate([bu[i][j][pl.ds(c * LP, L), :]
                              for c in range(g * 128 // L, (g + 1) * 128 // L)], axis=0)
             for j in range(7)], axis=1).astype(BF16)
        y = _nt(_wide(ccat, 2 * D), paced(h))
        x = xa_v[i][:, g * 128:(g + 1) * 128].astype(F32) * dcol[...]
        val["mxu"] = y[0:8]
        outt[i][g][0:D] = y + x

    def b3(i, g):
        u = _nn(_wide(wot, D), paced(pltpu.bitcast(ot[i][g], BF16)))
        val["mxu"] = u[0:8]
        outt[i][g][D:2 * D] = u

    def emit(i, g, j):
        t = i * G + g
        v = outt[i][g][j * 128:(j + 1) * 128].T
        last["emit"] = v[120:128]
        for p, (t0, nt, j0, nj) in enumerate(PIECES):
            if t0 <= t < t0 + nt and j0 <= j < j0 + nj:
                out_v[p][(t - t0) * 128:(t - t0 + 1) * 128, (j - j0) * 128:(j - j0 + 1) * 128] = v

    def send(p):
        copies[f"o{p}"].start()
        r0 = PIECES[p][1] * 128
        out_v[p][r0:r0 + 16, 0:128] = jnp.zeros((16, 128), F32)
        last["send"] = out_v[p][r0 + 4:r0 + 12, 0:128]

    def calls(f, *ranges):
        out = [()]
        for r in ranges:
            out = [a + (v,) for a in out for v in r]
        return [functools.partial(f, *a) for a in out]

    mxu, at, end, now = [], {}, {}, 0
    for name in ORDER.split():
        kind, i, gs = name[0], int(name[1]), [int(c) for c in name[2:]] or range(G)
        cost, fs = {"A": (512, calls(a1, [i], (6, 0, 3, 1, 4, 2, 5) if i else (0, 1, 2, 6, 3, 4, 5))),
                    "B": (448, calls(b1, [i], range(3), gs)),
                    "Y": (784, calls(a3, [i], gs)),
                    "O": (448, calls(b3, [i], gs))}[kind]
        at.setdefault(name[:2], now)
        for f in fs:
            mxu.append((now, now + cost, f))
            now += cost
            end[(kind,) + f.args] = now
    side = []

    def run(t0, pace, fs, deadline=None):
        side.extend((t0 + n * pace, f) for n, f in enumerate(fs))
        assert deadline is None or side[-1][0] < deadline, (fs[-1], side[-1][0], deadline)
        return side[-1][0] + pace

    scan = lambda i: calls(a2, [i], range(4), (0, 1), range(0, L, SCAN_STEP))
    run(at["A0"] + 2560, 100, calls(xt, [1], range(4)), at["A1"])
    run(at["A1"] + 1536, 200, calls(prep_wqkv, range(4)), at["B0"])
    run(at["A1"], 103, scan(0))
    run(at["B0"], 120, scan(1))
    run(at["A2"] - 300, 80, calls(prep_c, range(4), range(0, D, 64)), at["Y0"])
    run(at["Y1"] - 300, 500, calls(prep_wo, range(4)), at["O0"])
    run(at["A2"] - 1700, 200, calls(xt, [2], range(4)), at["A2"])
    run(at["B2"] + 500, 200, calls(xt, [3], range(4)), at["A3"])
    run(at["B2"], 120, scan(2), at["Y2"])
    run(at["B3"] + 1800, 110, scan(3), at["Y3"])
    t1 = 0
    for i in range(NB):
        run(end["A", i, 6], 0, [functools.partial(swap, i)])
        for n in range(3):
            t0 = run(end["B", i, n, G - 1], 50, calls(restack, [i], [n], range(NDP)))
        sc, bl = calls(scores, [i], range(0, 128, 8)), calls(blend, [i], range(0, 128, 8))
        t1 = run(max(t0 - 2 * ATT, t1), ATT,
                 sc[:AHEAD] + [f for pair in zip(sc[AHEAD:], bl) for f in pair] + bl[-AHEAD:])
        run(t1, 50, calls(unstack, [i], range(NDP)), at[f"O{i}"])
        for g in range(G):
            run(end["Y", i, g], 50, calls(emit, [i], [g], range(3)))
            run(end["O", i, g], 50, calls(emit, [i], [g], range(3, 7)))
    for p, (t0, nt, j0, nj) in enumerate(PIECES[:-1]):
        i, g = divmod(t0 + nt - 1, G)
        j = j0 + nj
        t1 = end["Y", i, g] + 50 * j if j <= 3 else end["O", i, g] + 50 * (j - 3)
        run(t1 - 1, 0, [functools.partial(send, p)])
    side.sort(key=lambda e: e[0])
    points = {at["A0"] + 1024: "b4 b1 b2 b3",
              at["A0"] + 2560: "xa1",
              at["A1"] + 1536: "wqkv xb0",
              at["B1"]: "xb1 cre cim wo xa2 xb2 xa3 xb3"}

    dma("v0 v1 v2 v3 xa0 b0 " + " ".join(points.values()), "v0 v1 v2 v3")
    prep_lambda()
    prep_skip()
    dma(wait="xa0")
    for f in calls(xt, [0], range(4)):
        f()
    dma(wait="b0")
    n = 0
    for t, stop, f in mxu:
        dma(wait=points.get(t, ""))
        f()
        while n < len(side) and side[n][0] < stop:
            side[n][1]()
            n += 1
    for _, f in side[n:]:
        f()
    dma(f"o{len(PIECES) - 1}", " ".join(f"o{p}" for p in range(len(PIECES))))


@jax.jit
def pallas_concat_heads__ssm_conv_s5__sliding_local_dilated__prompt_kernel(
    A_x: jax.Array,
    A_Lambda_re: jax.Array,
    A_Lambda_im: jax.Array,
    A_B_re: jax.Array,
    A_B_im: jax.Array,
    A_C_re: jax.Array,
    A_C_im: jax.Array,
    A_log_dt: jax.Array,
    A_Dskip: jax.Array,
    B_x: jax.Array,
    B_wqkv: jax.Array,
    B_wo: jax.Array,
):
    hbm = pl.BlockSpec(memory_space=pl.ANY)
    out = pl.pallas_call(
        _kernel,
        in_specs=[hbm] * 12,
        out_specs=hbm,
        out_shape=jax.ShapeDtypeStruct((S, 2 * D), F32),
        scratch_shapes=[
            [pltpu.VMEM((D,), BF16)] * 4,
            [pltpu.VMEM((D, T), BF16)] * NB,
            [pltpu.VMEM((D, T), BF16)] * NB,
            pltpu.VMEM((2 * D, D), BF16),
            pltpu.VMEM((D, D), BF16),
            pltpu.VMEM((D, D), BF16),
            pltpu.VMEM((D, 3 * D), BF16),
            pltpu.VMEM((D, D), BF16),
            [pltpu.VMEM((nt * 128 + 16, nj * 128), F32) for _, nt, _, nj in PIECES],
            pltpu.VMEM((4, 3 * D // 2, 128), U32),
            pltpu.VMEM((4, D // 2, 128), U32),
            pltpu.VMEM((7, D // 2, 128), U32),
            pltpu.VMEM((D, 128), F32),
            pltpu.VMEM((8, 4, 8, 128), F32),
            pltpu.VMEM((2, 4, 8, 128), F32),
            pltpu.VMEM((4, D, 128), F32),
            pltpu.SemaphoreType.DMA((13 + 2 * NB,)),
            pltpu.SemaphoreType.DMA((len(PIECES),)),
            [[pltpu.VMEM((8 * LP, 128), F32)] * 8] * NB,
            [pltpu.VMEM((G, 3 * D, 128), F32)] * NB,
            [pltpu.VMEM((NDP, 128, 128), F32)] * NB,
            [pltpu.VMEM((NDP, HALO + 128, 128), F32)] * NB,
            [pltpu.VMEM((NDP, HALO + 128, 128), F32)] * NB,
            [pltpu.VMEM((G, D // 2, 128), U32)] * NB,
            [pltpu.VMEM((4, T // 2, 128), U32)] * NB,
            [[pltpu.VMEM((2 * D, 128), F32)] * G] * NB,
        ],
        compiler_params=pltpu.CompilerParams(vmem_limit_bytes=110 << 20, flags={"XLA_TPU_FORCE_LP_LLO_SCHEDULER": True}),
        name="s5_dilated_attn",
    )(A_Lambda_re, A_Lambda_im, A_log_dt, A_Dskip,
      jnp.swapaxes(A_x[0], 0, 1), jnp.swapaxes(B_x[0], 0, 1),
      A_B_re, A_B_im, A_C_re, A_C_im, B_wqkv, B_wo)
    return out[None]
```

```python
import functools

import jax
import jax.numpy as jnp
from jax import lax
import jax.experimental.pallas as pl
import jax.experimental.pallas.tpu as pltpu

F32 = jnp.float32
BF16 = jnp.bfloat16
U32 = jnp.uint32

S = 2048
D = 448
H = 16
DH = D // H
W = 8
DIL = 2
T = 512
NB = S // T
G = T // 128
L = T // 8
LP = L + 1
NDP = DH // 2
HALO = 16
LOG2E = 1.4426950408889634
SCAN_STEP = 16
KT = ((0, 128), (128, 128), (256, 128), (384, 64))

ORDER = ("H0 H1 A0 A1 B0 B1 A2 Y0 Y1 O0 O1 B2 A3 B3 Y20 O20 Y21 O21 Y22 O22 Y23 O23 "
         "Y30 Y31 O30 O31 Y32 O32 O33 Y33")
PIECES = (((0, 8, 0, 7),) + tuple((t, 1, 0, 7) for t in range(8, 12))
          + tuple((t, 1, j, n) for t in range(12, 15) for j, n in ((0, 3), (3, 4)))
          + ((15, 1, 4, 3), (15, 1, 0, 2), (15, 1, 2, 2)))
LAG, LAG_OUT, LAG_OUT_LAST = 3000, 1500, 500


def _nt(a, b):
    return lax.dot_general(a, b, (((1,), (1,)), ((), ())), preferred_element_type=F32)


def _nn(a, b):
    return jnp.dot(a, b, preferred_element_type=F32)


def _cmul(ar, ai, br, bi):
    return ar * br - ai * bi, ar * bi + ai * br


def _pack(x):
    return pltpu.bitcast(x.astype(BF16), U32)


def _wide(ref, width):
    n = -(-width // 128)
    x = jnp.concatenate([pltpu.bitcast(ref[j], BF16) for j in range(n)], axis=1)
    return x[:, 0:width]


def _head_minor(ref, base, dp):
    even = ref[pl.ds(base + dp, 8, stride=DH), :]
    odd = ref[pl.ds(base + dp + NDP, 8, stride=DH), :]
    return [(even & 0xFFFF) | (odd << 16), (even >> 16) | ((odd >> 16) << 16)]


def _calls(f, *ranges):
    args = [()]
    for r in ranges:
        args = [a + (v,) for a in args for v in r]
    return [functools.partial(f, *a) for a in args]


def _kernel(lre_hbm, lim_hbm, ldt_hbm, dsk_hbm, xa_hbm, xb_hbm, bre_hbm, bim_hbm,
            cre_hbm, cim_hbm, wqkv_hbm, wo_hbm, out_hbm,
            vec, xa_v, xb_v, bcat, cre_v, cim_v, wqkv_v, wo_v, out_v,
            wqt, wot, ccat, dcol, lam, coef, wqf, wof, sems,
            bu, stage, qs, ks, vs, ot, xat, outt):
    lane = lax.broadcasted_iota(jnp.int32, (8, 128), 1)
    sub = lax.broadcasted_iota(jnp.int32, (8, 128), 0)

    cols = lambda i: pl.ds(i * T, T)
    groups = [
        list(zip((lre_hbm, lim_hbm, ldt_hbm, dsk_hbm), vec)),
        [(xa_hbm.at[:, 0:T // 2], xa_v[0].at[:, 0:T // 2])],
        [(bre_hbm.at[0:256], bcat.at[0:256])],
        [(xa_hbm.at[:, T // 2:T], xa_v[0].at[:, T // 2:T]),
         (bre_hbm.at[256:384], bcat.at[256:384])],
        [(bim_hbm.at[0:384], bcat.at[384:768]),
         (bre_hbm.at[384:448], bcat.at[768:832]), (bim_hbm.at[384:448], bcat.at[832:896])],
        [(xa_hbm.at[:, cols(1)], xa_v[1])],
        [(wqkv_hbm, wqkv_v), (xb_hbm.at[:, cols(0)], xb_v[0])],
        [(cre_hbm, cre_v), (cim_hbm, cim_v), (wo_hbm, wo_v)]
        + [(xb_hbm.at[:, cols(i)], xb_v[i]) for i in range(1, NB)]
        + [(xa_hbm.at[:, cols(i)], xa_v[i]) for i in range(2, NB)],
    ]
    loads = [[pltpu.make_async_copy(src, dst, sems.at[n]) for src, dst in group]
             for n, group in enumerate(groups)]
    stores = [pltpu.make_async_copy(
        out_v[p].at[0:nt * 128],
        out_hbm.at[pl.ds(t0 * 128, nt * 128), pl.ds(j0 * 128, nj * 128)], sems.at[len(groups)])
        for p, (t0, nt, j0, nj) in enumerate(PIECES)]

    def wait(copies):
        for c in copies:
            c.wait()

    val, last, history = {}, {}, {}

    def tie(dep, x):
        n = x.shape[1]
        dep = dep if dep.dtype == x.dtype else pltpu.bitcast(dep, x.dtype)
        return jnp.concatenate(
            [jnp.where(val["never"][:, 0:n], dep[:, 0:n], x[r:r + 8])
             for r in range(0, x.shape[0], 8)], axis=0)

    def after(stream, x):
        return tie(last[stream], x) if stream in last else x

    def released(x):
        return tie(val["mxu"], x)

    def paced(rhs, offset=0):
        deps = []
        for k, log in history.items():
            lag = (LAG if k not in ("emit", "send") else
                   LAG_OUT_LAST if val["now"] >= at["Y3"] else LAG_OUT)
            ready = [v for t, v in log if t <= val["now"] + offset - lag]
            if ready:
                deps.append(ready[-1])
                del log[:len(ready)]
        if not deps:
            return rhs
        head = pltpu.bitcast(rhs[0:16, 0:128], U32)
        for v in deps:
            head = tie(v, head)
        head = pltpu.bitcast(head, BF16)
        if rhs.shape[1] > 128:
            head = jnp.concatenate([head, rhs[0:16, 128:]], axis=1)
        return jnp.concatenate([head, rhs[16:]], axis=0)

    def prep_lambda():
        lr = vec[0][...].astype(F32).reshape(1, D)
        li = vec[1][...].astype(F32).reshape(1, D)
        dt = jnp.exp(vec[2][...].astype(F32).reshape(1, D)).astype(BF16).astype(F32)
        mag = jnp.exp(dt * lr)
        ar = mag * jnp.cos(dt * li)
        ai = mag * jnp.sin(dt * li)
        nr, ni = ar - 1.0, ai
        big = jnp.abs(lr) >= jnp.abs(li)
        r = jnp.where(big, li / lr, lr / li)
        den = jnp.where(big, lr + li * r, lr * r + li)
        fr = 2.0 * jnp.where(big, nr + ni * r, nr * r + ni) / den
        fi = 2.0 * jnp.where(big, ni - nr * r, ni * r - nr) / den
        for j in range(4):
            if j < 3:
                pr, pi, qr, qi = (v[:, j * 128:(j + 1) * 128] for v in (ar, ai, fr, fi))
            else:
                pr = jnp.concatenate([ar[:, 384:], ar[:, 384:]], axis=1)
                pi = jnp.concatenate([ai[:, 384:], -ai[:, 384:]], axis=1)
                qr = jnp.concatenate([fr[:, 384:], -fr[:, 384:]], axis=1)
                qi = jnp.concatenate([fi[:, 384:], fi[:, 384:]], axis=1)
            coef[0, j], coef[1, j] = jnp.broadcast_to(qr, (8, 128)), jnp.broadcast_to(qi, (8, 128))
            pr = jnp.broadcast_to(pr, (8, 128))
            pi = jnp.broadcast_to(pi, (8, 128))
            lam[0, j], lam[1, j] = pr, pi
            for _ in range(L.bit_length() - 1):
                pr, pi = _cmul(pr, pi, pr, pi)
            for k in range(3):
                lam[2 + 2 * k, j], lam[3 + 2 * k, j] = pr, pi
                pr, pi = _cmul(pr, pi, pr, pi)
        a = jnp.broadcast_to(lr[:, 0:128], (8, 128))
        b = jnp.broadcast_to(li[:, 0:128], (8, 128))
        val["never"] = (a > b) & (b > a)

    def prep_skip():
        dsk = jnp.broadcast_to(vec[3][...].astype(F32).reshape(1, D), (128, D))
        dcol[...] = dsk.T

    def prep_c(j, r0):
        tile = slice(KT[j][0], KT[j][0] + KT[j][1])
        for r in range(r0, r0 + 64, 16):
            cr, ci = cre_v[r:r + 16, tile].astype(F32), cim_v[r:r + 16, tile].astype(F32)
            if j == 3:
                cr, ci = jnp.concatenate([cr, ci], axis=1), jnp.concatenate([ci, cr], axis=1)
            fr = after("prep", coef[0, j])
            fi = after("prep", coef[1, j])
            if r == r0:
                fr = released(fr)
            fr, fi = (jnp.concatenate([v, v], axis=0) for v in (fr, fi))
            half = slice(r // 2, r // 2 + 8)
            ccat[6 if j == 3 else j, half] = done = _pack(cr * fr - ci * fi)
            if j < 3:
                ccat[3 + j, half] = done = _pack(-(cr * fi + ci * fr))
            last["prep"] = done

    def prep_wqkv(n, j):
        k0, wd = KT[j]
        c0, c1 = ((0, 512), (512, 896), (896, 3 * D))[n]
        w = wqkv_v[k0:k0 + wd, c0:c1]
        if n:
            w = pltpu.bitcast(w, U32)
            w = jnp.concatenate([released(w[:, 0:128]), w[:, 128:]], axis=1)
            w = pltpu.bitcast(w, BF16)
        if wd < 128:
            w = jnp.concatenate([w, jnp.zeros((128 - wd, c1 - c0), BF16)], axis=0)
        wqf[j][c0 // 2:c1 // 2] = _pack(w.T)
        for dp in range(NDP):
            wqt[j, pl.ds(n * D // 2 + dp * H, H)] = jnp.concatenate(
                _head_minor(wqf[j], n * D // 2, dp), axis=0)

    def prep_wo(j):
        n0, wd = KT[j]
        if wd < 128:
            wof[j][:, wd:] = jnp.zeros((D // 2, 128 - wd), U32)
        wof[j][:, 0:wd] = released(pltpu.bitcast(wo_v[:, n0:n0 + wd], U32))
        for k, (k0, kw) in enumerate(KT):
            rows = [pltpu.bitcast(v, BF16)
                    for dp in range(k0 // (2 * H), (k0 + kw) // (2 * H))
                    for v in _head_minor(wof[j], 0, dp)]
            if kw < 128:
                rows.append(jnp.zeros((128 - kw, 128), BF16))
            t = _pack(jnp.concatenate(rows, axis=0).T[0:wd])
            wot[k, n0 // 2:(n0 + wd) // 2] = t
        last["prep"] = t[0:8]

    def xt(i, s0):
        x = xa_v[i][:, s0:s0 + T // 2]
        x = _pack(jnp.concatenate([x, jnp.zeros((512 - D, T // 2), BF16)], axis=0).T)
        for j in range(4):
            xat[i][j, s0 // 2:s0 // 2 + T // 4] = x[:, j * 128:(j + 1) * 128]

    def a1(i, j, s0=0, ns=T):
        x = _wide(xat[i].at[:, s0 // 2:(s0 + ns) // 2], D)
        u = _nt(x, paced(bcat[j * 128:(j + 1) * 128]))
        val["mxu"] = u[0:8]
        for c in range(ns // L):
            bu[i][j][pl.ds((s0 // L + c) * LP, L), :] = u[c * L:(c + 1) * L]

    def swap(i):
        for c in range(8):
            bu[i][7][pl.ds(c * LP, L), :] = pltpu.roll(bu[i][6][pl.ds(c * LP, L), :], 64, 1)

    carry = [(0.0, 0.0)] * 4
    state = [None] * 4

    def a2(i, j, second, r0):
        jr, ji = (j, j + 3) if j < 3 else (6, 7)
        pr, pi = lam[0, j], lam[1, j]
        if second and r0 == 0:
            hr, hi = state[j]
            cr, ci = carry[j]
            hr = pltpu.roll(jnp.where(sub == 7, cr, hr), 1, 0)
            hi = pltpu.roll(jnp.where(sub == 7, ci, hi), 1, 0)
            for k in range(3):
                sr = jnp.where(sub >= (1 << k), pltpu.roll(hr, 1 << k, 0), 0.0)
                si = jnp.where(sub >= (1 << k), pltpu.roll(hi, 1 << k, 0), 0.0)
                mr, mi = _cmul(lam[2 + 2 * k, j], lam[3 + 2 * k, j], sr, si)
                hr, hi = hr + mr, hi + mi
            state[j] = hr, hi
        for r in range(r0, r0 + SCAN_STEP):
            ur = bu[i][jr][pl.ds(r, 8, stride=LP), :]
            ui = bu[i][ji][pl.ds(r, 8, stride=LP), :]
            if r == 0 and not second:
                state[j] = released(after("scan", ur)), after("scan", ui)
                continue
            mr, mi = _cmul(pr, pi, *state[j])
            state[j] = hr, hi = mr + ur, mi + ui
            if second:
                bu[i][jr][pl.ds(r, 8, stride=LP), :] = hr
                if j < 3:
                    bu[i][ji][pl.ds(r, 8, stride=LP), :] = hi
        if second and r0 + SCAN_STEP == L:
            carry[j] = state[j]
        last["scan"] = state[j][0]

    def a3(i, g):
        h = jnp.concatenate(
            [jnp.concatenate([bu[i][j][pl.ds(c * LP, L), :]
                              for c in range(g * 128 // L, (g + 1) * 128 // L)], axis=0)
             for j in range(7)], axis=1).astype(BF16)
        h = jnp.concatenate([paced(h[:, 0:512]), paced(h[:, 512:], 400)], axis=1)
        y = _nt(_wide(ccat, 2 * D), h)
        x = xa_v[i][:, g * 128:(g + 1) * 128].astype(F32) * dcol[...]
        val["mxu"] = y[0:8]
        outt[i][g][0:D] = y + x

    def b1(i, n, g):
        w = _wide(wqt.at[:, n * D // 2:(n + 1) * D // 2], D)
        u = _nn(w, paced(xb_v[i][:, g * 128:(g + 1) * 128]))
        val["mxu"] = u[0:8]
        stage[i][g, n * D:(n + 1) * D] = u

    def restack(i, which, dp):
        dst = (qs, ks, vs)[which]
        pieces = [stage[i][g, pl.ds(which * D + (2 * dp + e) * H, H), :]
                  for e in range(2) for g in range(G)]
        t = jnp.concatenate(pieces, axis=0).T
        last["xlu"] = t[120:128]
        if which == 0:
            dst[i][dp] = t
            return
        dst[i][dp, HALO:] = t
        if i == 0:
            first = jnp.broadcast_to(t[0:1], (HALO, 128))
        else:
            first = pltpu.roll(dst[i - 1][dp, 128:], 128 - (G - 1) * H, 1)
        half = lax.broadcasted_iota(jnp.int32, (HALO, 128), 1) % 64
        dst[i][dp, 0:HALO] = jnp.where(half < H, first, pltpu.roll(t[128 - HALO:], H, 1))

    probs = {}

    def scores(i, r0):
        lg = []
        for w in range(W):
            for dp in range(NDP):
                t = qs[i][dp, r0:r0 + 8] * ks[i][dp, pl.ds(HALO + r0 - DIL * w, 8), :]
                a = after("qk", t) if dp == 0 else a + t
                if dp == 0 and w == 0:
                    a = after("pv", a)
            last["qk"] = a
            a = a + pltpu.roll(a, 64, 1)
            if i == 0 and r0 - DIL * w < 0:
                bad = ((lane % 64) < H) & (sub + (r0 - DIL * w) < 0)
                a = jnp.where(bad, -1e9 * DH ** 0.5, a)
            lg.append(a)
        m = functools.reduce(jnp.maximum, lg)
        ex = [jnp.exp2((x - m) * (DH ** -0.5 * LOG2E)) for x in lg]
        inv = 1.0 / functools.reduce(jnp.add, ex)
        probs[i, r0] = [x * inv for x in ex]

    def blend(i, r0):
        p = probs.pop((i, r0))
        for dp in range(NDP):
            o = after("pv", p[0] * vs[i][dp, pl.ds(HALO + r0, 8), :])
            for w in range(1, W):
                o = o + p[w] * vs[i][dp, pl.ds(HALO + r0 - DIL * w, 8), :]
            last["pv"] = o
            qs[i][dp, r0:r0 + 8] = o

    def unstack(i, dp):
        t = qs[i][dp].T
        last["xlu"] = t[120:128]
        for e in range(2):
            for g in range(G):
                ot[i][g, pl.ds((2 * dp + e) * H // 2, H // 2), :] = _pack(
                    t[(e * G + g) * H:(e * G + g + 1) * H])

    def b3(i, g):
        u = _nn(_wide(wot, D), paced(pltpu.bitcast(ot[i][g], BF16)))
        val["mxu"] = u[0:8]
        outt[i][g][D:2 * D] = u

    def emit(i, g, j):
        t = i * G + g
        v = outt[i][g][j * 128:(j + 1) * 128].T
        last["emit"] = v[120:128]
        for p, (t0, nt, j0, nj) in enumerate(PIECES):
            if t0 <= t < t0 + nt and j0 <= j < j0 + nj:
                out_v[p][(t - t0) * 128:(t - t0 + 1) * 128, (j - j0) * 128:(j - j0 + 1) * 128] = v

    def send(p):
        stores[p].start()
        r0 = PIECES[p][1] * 128
        out_v[p][r0:r0 + 16, 0:128] = jnp.zeros((16, 128), F32)
        last["send"] = out_v[p][r0 + 4:r0 + 12, 0:128]

    mxu, at, end, now = [], {}, {}, 0
    for name in ORDER.split():
        kind, i, gs = name[0], int(name[1]), [int(c) for c in name[2:]] or range(G)
        cost, fs = {"A": (512, _calls(a1, [i], (6, 0, 3, 1, 4, 2, 5) if i else (6, 3, 4, 5))),
                    "H": (256, _calls(a1, [0], range(3), [i * T // 2], [T // 2])),
                    "B": (448, _calls(b1, [i], range(3), gs)),
                    "Y": (784, _calls(a3, [i], gs)),
                    "O": (448, _calls(b3, [i], gs))}[kind]
        at.setdefault(name[:2], now)
        for f in fs:
            mxu.append((now, now + cost, f))
            now += cost
            end[(kind,) + f.args] = now
    side = []

    def run(t0, pace, fs, deadline=None):
        side.extend((t0 + n * pace, f) for n, f in enumerate(fs))
        assert deadline is None or side[-1][0] < deadline
        return side[-1][0] + pace

    scan = lambda i: _calls(a2, [i], range(4), (0, 1), range(0, L, SCAN_STEP))
    halves = (0, T // 2)
    t_wqkv = at["A1"] + 2048
    run(at["H1"] - 256, 0, _calls(xt, [0], halves[1:]), at["H1"])
    run(at["A0"] + 1024, 100, _calls(xt, [1], halves), at["A1"])
    run(t_wqkv, 200, _calls(prep_wqkv, [0], range(4)), at["B0"])
    run(at["B0"] - 300, 250, _calls(prep_wqkv, [1], range(4)), end["B", 0, 0, G - 1])
    run(end["B", 0, 0, G - 1] - 300, 250, _calls(prep_wqkv, [2], range(4)), end["B", 0, 1, G - 1])
    run(at["A1"], 100, scan(0)[:20], t_wqkv)
    run(at["B0"], 115, scan(0)[20:] + scan(1), at["Y0"])
    run(at["A2"] - 500, 80, _calls(prep_c, range(4), range(0, D, 64)), at["Y0"])
    run(at["Y1"] - 300, 400, _calls(prep_wo, range(4)), at["O0"])
    run(at["A2"] - 1700, 400, _calls(xt, [2], halves), at["A2"])
    run(at["B2"] + 500, 400, _calls(xt, [3], halves), at["A3"])
    run(at["B2"], 120, scan(2), at["Y2"])
    run(at["B3"] + 2400, 110, scan(3), at["Y3"])
    t1 = 0
    for i in range(NB):
        run(end["A", i, 6], 0, _calls(swap, [i]))
        for n in range(3):
            t0 = run(end["B", i, n, G - 1], 48, _calls(restack, [i], [n], range(NDP)))
        sc, bl = _calls(scores, [i], range(0, 128, 8)), _calls(blend, [i], range(0, 128, 8))
        t1 = run(max(t0 - 240, t1), 120,
                 sc[:1] + [f for pair in zip(sc[1:], bl) for f in pair] + bl[-1:])
        run(t1, 50, _calls(unstack, [i], range(NDP)), at[f"O{i}"])
        for g in range(G):
            ty, to = end["Y", i, g], end["O", i, g]
            ja = 3 if ty < to else 4
            run(ty, 50, _calls(emit, [i], [g], range(ja)))
            run(to, 50, _calls(emit, [i], [g], range(ja, 7)))
    emitted = {f.args: t for t, f in side if f.func is emit}
    for p, (t0, nt, j0, nj) in enumerate(PIECES[:-1]):
        tiles = [(*divmod(t, G), j) for t in range(t0, t0 + nt) for j in range(j0, j0 + nj)]
        run(max(emitted[k] for k in tiles), 0, _calls(send, [p]))
    side.sort(key=lambda e: e[0])
    arrivals = {at["H1"] - 256: loads[3], at["A0"]: loads[4], at["A0"] + 1024: loads[5],
                t_wqkv: loads[6], at["B1"]: loads[7]}

    for group in loads:
        for c in group:
            c.start()
    wait(loads[0])
    prep_lambda()
    prep_skip()
    wait(loads[1])
    xt(0, 0)
    wait(loads[2])
    n = 0
    for t, stop, f in mxu:
        wait(arrivals.get(t, ()))
        val["now"] = t
        f()
        while n < len(side) and side[n][0] < stop:
            before = dict(last)
            side[n][1]()
            for k, v in last.items():
                if before.get(k) is not v:
                    history.setdefault(k, []).append((side[n][0], v))
            n += 1
    for _, f in side[n:]:
        f()
    stores[-1].start()
    wait(stores)


@jax.jit
def pallas_concat_heads__ssm_conv_s5__sliding_local_dilated__prompt_kernel(
    A_x: jax.Array,
    A_Lambda_re: jax.Array,
    A_Lambda_im: jax.Array,
    A_B_re: jax.Array,
    A_B_im: jax.Array,
    A_C_re: jax.Array,
    A_C_im: jax.Array,
    A_log_dt: jax.Array,
    A_Dskip: jax.Array,
    B_x: jax.Array,
    B_wqkv: jax.Array,
    B_wo: jax.Array,
):
    hbm = pl.BlockSpec(memory_space=pl.ANY)
    out = pl.pallas_call(
        _kernel,
        in_specs=[hbm] * 12,
        out_specs=hbm,
        out_shape=jax.ShapeDtypeStruct((S, 2 * D), F32),
        scratch_shapes=[
            [pltpu.VMEM((D,), BF16)] * 4,
            [pltpu.VMEM((D, T), BF16)] * NB,
            [pltpu.VMEM((D, T), BF16)] * NB,
            pltpu.VMEM((2 * D, D), BF16),
            pltpu.VMEM((D, D), BF16),
            pltpu.VMEM((D, D), BF16),
            pltpu.VMEM((D, 3 * D), BF16),
            pltpu.VMEM((D, D), BF16),
            [pltpu.VMEM((nt * 128 + 16, nj * 128), F32) for _, nt, _, nj in PIECES],
            pltpu.VMEM((4, 3 * D // 2, 128), U32),
            pltpu.VMEM((4, D // 2, 128), U32),
            pltpu.VMEM((7, D // 2, 128), U32),
            pltpu.VMEM((D, 128), F32),
            pltpu.VMEM((8, 4, 8, 128), F32),
            pltpu.VMEM((2, 4, 8, 128), F32),
            [pltpu.VMEM((3 * D // 2, 128), U32)] * 4,
            [pltpu.VMEM((D // 2, 128), U32)] * 4,
            pltpu.SemaphoreType.DMA((9,)),
            [[pltpu.VMEM((8 * LP, 128), F32)] * 8] * NB,
            [pltpu.VMEM((G, 3 * D, 128), F32)] * NB,
            [pltpu.VMEM((NDP, 128, 128), F32)] * NB,
            [pltpu.VMEM((NDP, HALO + 128, 128), F32)] * NB,
            [pltpu.VMEM((NDP, HALO + 128, 128), F32)] * NB,
            [pltpu.VMEM((G, D // 2, 128), U32)] * NB,
            [pltpu.VMEM((4, T // 2, 128), U32)] * NB,
            [[pltpu.VMEM((2 * D, 128), F32)] * G] * NB,
        ],
        compiler_params=pltpu.CompilerParams(
            vmem_limit_bytes=110 << 20, flags={"XLA_TPU_FORCE_LP_LLO_SCHEDULER": True}),
        name="s5_dilated_attn",
    )(A_Lambda_re, A_Lambda_im, A_log_dt, A_Dskip,
      jnp.swapaxes(A_x[0], 0, 1), jnp.swapaxes(B_x[0], 0, 1),
      A_B_re, A_B_im, A_C_re, A_C_im, B_wqkv, B_wo)
    return out[None]
```
